```python
import jax
import jax.numpy as jnp

def _softmax(x, axis=-1):
    return jax.nn.softmax(x, axis=axis)
def _gelu(x):
    return jax.nn.gelu(x, approximate=True)
def _silu(x):
    return jax.nn.silu(x)
def _sigmoid(x):
    return jax.nn.sigmoid(x)
def _layernorm(x, axis=-1, eps=1e-5):
    m = jnp.mean(x, axis=axis, keepdims=True)
    v = jnp.var(x, axis=axis, keepdims=True)
    return (x - m) / jnp.sqrt(v + eps)
def _scatter_add(tgt, idx, src, axis=0):
    return tgt.at[idx].add(src)
def _segment_sum(src, seg, n):
    return jax.ops.segment_sum(src, seg, n)
class _Rng:
    def __init__(self, key):
        self._k = key
    def _next(self):
        self._k, sub = jax.random.split(self._k)
        return sub
    def normal(self, shape):
        return jax.random.normal(self._next(), shape, dtype=jnp.bfloat16)
    def randint(self, lo, hi, shape):
        return jax.random.randint(self._next(), shape, lo, hi, dtype=jnp.int32)
    def uniform(self, shape, lo=0.0, hi=1.0):
        return jax.random.uniform(self._next(), shape, jnp.bfloat16, lo, hi)
    def permutation(self, n):
        return jax.random.permutation(self._next(), n)


kernel_name = 'interleave_layers__sliding_local_dilated__mixer_token_mlp__prompt'

def setup_inputs():
    _rng = _Rng(jax.random.key(int.from_bytes(__import__("os").urandom(4), "little")))
    _w = (lambda a: (lambda t: t.astype(jnp.bfloat16) if jnp.issubdtype(t.dtype, jnp.floating) else t)(jnp.asarray(a)))
    def _A_setup():
        B, S, D = 1, 2048, 1024
        return {
            "x": _w((lambda *s: _rng.normal(s) * 0.05)(B, S, D)),
            "wqkv": _w((lambda *s: _rng.normal(s) * 0.05)(D, 3 * D)),
            "wo": _w((lambda *s: _rng.normal(s) * 0.05)(D, D)),
        }
    _A_in = _A_setup()

    def _B_setup():
        B, S, D, F = 1, 2048, 1024, 3584
        return {
            "x": _w((lambda *s: _rng.normal(s) * 0.05)(B, S, D)),
            "w1": _w((lambda *s: _rng.normal(s) * 0.05)(S, F) * (S ** -0.5)),
            "b1": _w((lambda *s: _rng.normal(s) * 0.05)(F) * 0.02),
            "w2": _w((lambda *s: _rng.normal(s) * 0.05)(F, S) * (F ** -0.5)),
            "b2": _w((lambda *s: _rng.normal(s) * 0.05)(S) * 0.02),
        }
    _B_in = _B_setup()

    return {
        "A_x": _A_in["x"],
        "A_wqkv": _A_in["wqkv"],
        "A_wo": _A_in["wo"],
        "B_x": _B_in["x"],
        "B_w1": _B_in["w1"],
        "B_b1": _B_in["b1"],
        "B_w2": _B_in["w2"],
        "B_b2": _B_in["b2"],
    }

def reference(A_x, A_wqkv, A_wo, B_x, B_w1, B_b1, B_w2, B_b2):
    def _A_ref(x, wqkv, wo):
        B, S, D = x.shape
        H = 32; Dh = D // H
        W, dil = 8, 2
        qkv = (lambda x, *d: x.transpose(*d))((x @ wqkv).reshape(B, S, 3, H, Dh), 2, 0, 3, 1, 4)
        q, k, v = qkv[0], qkv[1], qkv[2]
        scale = Dh ** -0.5
        pos = jnp.arange(S)
        off = jnp.arange(W) * dil
        idx = pos[:, None] - off[None, :]
        mask = idx >= 0
        idx_c = jnp.where(mask, idx, 0).reshape(-1)
        kg = k[:, :, idx_c, :].reshape(B, H, S, W, Dh)
        vg = v[:, :, idx_c, :].reshape(B, H, S, W, Dh)
        logits = jnp.einsum("bhsd,bhswd->bhsw", q, kg) * scale
        logits = jnp.where(mask[None, None, :, :], logits, -1e9)
        attn = _softmax(logits, axis=-1)
        o = jnp.einsum("bhsw,bhswd->bhsd", attn, vg)
        return (lambda x, *d: x.transpose(*d))(o, 0, 2, 1, 3).reshape(B, S, D) @ wo

    def _B_ref(x, w1, b1, w2, b2):
        B, S, D = x.shape
        h = _layernorm(x, axis=-1)
        u = jnp.einsum("bsd,sf->bdf", h, w1) + b1
        u = _gelu(u)
        y = jnp.einsum("bdf,fs->bds", u, w2) + b2
        return (lambda x, *d: x.transpose(*d))(y, 0, 2, 1)

    x = A_x
    x = x + _A_ref(_layernorm(x, axis=-1), A_wqkv, A_wo)
    x = x + _B_ref(_layernorm(x, axis=-1), B_w1, B_b1, B_w2, B_b2)
    x = x + _A_ref(_layernorm(x, axis=-1), A_wqkv, A_wo)
    x = x + _B_ref(_layernorm(x, axis=-1), B_w1, B_b1, B_w2, B_b2)
    return x
```

```python
import jax
import jax.numpy as jnp
from jax import lax
import jax.experimental.pallas as pl
import jax.experimental.pallas.tpu as pltpu

S, D, F = 2048, 1024, 3584
NH, DH, WIN = 32, 32, 8
NB = S // 128
EPS = 1e-5
BF, F32, U32 = jnp.bfloat16, jnp.float32, jnp.uint32
NT = (((1,), (1,)), ((), ()))


def _perm_rows(ref_u32, lead, j):
    return pltpu.bitcast(ref_u32[lead, pl.ds(j, 64, stride=NB), :], BF)


def _ln(x, twice):
    m = jnp.mean(x, axis=0, keepdims=True)
    c = x - m
    v = jnp.mean(c * c, axis=0, keepdims=True)
    r = lax.rsqrt(v + EPS)
    if twice:
        r = r * lax.rsqrt(v * r * r + EPS)
    return (c * r).astype(BF)


def _gelu(x):
    return 0.5 * x * (1.0 + jnp.tanh(0.7978845608028654 * (x + 0.044715 * x * x * x)))


def _kernel(x_h, wqkv_h, wo_h, w1_h, b1_ref, w2_h, b2_ref, out_h,
            xs_u, wraw, woraw, w1s, w2raw, X, H, WT, WoT, w2t_u, KB, VB, Q, O, U, st, B1, B2, sems):
    xs, w1_u = xs_u.bitcast(BF), w1s.bitcast(U32)

    def col_copies(src, dst, lo, hi, sem):
        return [pltpu.make_async_copy(src.at[:, pl.ds(c * 128, 128)], dst.at[c], sems.at[sem])
                for c in range(lo, hi)]

    cp_x = col_copies(x_h, xs, 0, 8, 0)
    cp_w = [col_copies(wqkv_h, wraw, 8 * p, 8 * p + 8, 1 + p) for p in range(3)]
    cp_wo = [pltpu.make_async_copy(wo_h, woraw, sems.at[4])]
    cp_w1 = col_copies(w1_h, w1s, 0, F // 128, 5)
    cp_w2 = [pltpu.make_async_copy(w2_h, w2raw, sems.at[6])]
    for cp in cp_w[1] + cp_x + cp_w[2] + cp_w[0] + cp_wo + cp_w1 + cp_w2:
        cp.start()

    def wait(cps):
        for cp in cps:
            cp.wait()

    def prep_w(part, kc):
        rows = pl.ds(pl.multiple_of(kc * 128, 128), 128)
        for c in range(8):
            st[c * 128:(c + 1) * 128, :] = wraw[part * 8 + c, rows, :].astype(F32).T
        for g in range(4):
            for d in range(0, DH, 2):
                a = st[pl.ds(g * 256 + d, 8, stride=DH), :]
                b = st[pl.ds(g * 256 + d + 1, 8, stride=DH), :]
                r0 = g * 256 + d * 8
                WT[part, r0:r0 + 16, rows] = jnp.concatenate([a, b], axis=0).astype(BF)

    def prep_wo(c):
        cols = pl.ds(pl.multiple_of(c * 128, 128), 128)
        st[...] = woraw[:, cols].astype(F32)
        for k in range(8):
            g, d0 = k // 2, (k % 2) * 16
            blk = jnp.concatenate([st[pl.ds(g * 256 + d0 + d, 8, stride=DH), :] for d in range(16)], axis=0)
            WoT[cols, k * 128:(k + 1) * 128] = blk.T.astype(BF)

    def prep_w2(c):
        rows = pl.ds(pl.multiple_of(c * 128, 128), 128)
        for j in range(NB):
            w2t_u[c, j * 64:(j + 1) * 64, :] = pltpu.bitcast(w2raw[rows, j * 128:(j + 1) * 128].T, U32)

    def prep_x(j):
        xt = jnp.concatenate([_perm_rows(xs_u, c, j).T for c in range(8)], axis=0).astype(F32)
        X[j] = xt
        H[j] = _ln(xt, False)
        B2[j] = _perm_rows(xs_u, 8, j).T[0:16, :].astype(F32)[0:8, :]

    B1[...] = jnp.broadcast_to(b1_ref[...].astype(F32).reshape(1, F), (8, F))
    b2 = b2_ref[...].astype(F32).reshape(1, S)
    for c in range(NB):
        xs_u[8, c * 64:(c + 1) * 64, :] = pltpu.bitcast(
            jnp.broadcast_to(b2[:, c * 128:(c + 1) * 128], (128, 128)).T.astype(BF), U32)

    def loop(n, fn, lo=0):
        def body(i, c):
            fn(i)
            return c
        lax.fori_loop(lo, n, body, 0)

    def proj(part, t):
        h = jnp.concatenate([H[2 * t], H[2 * t + 1]], axis=1)
        return jnp.dot(WT[part], h, preferred_element_type=F32)

    def proj_kv(part, dst, t):
        r = proj(part, t)
        dst[2 * t + WIN - 1] = r[:, :128]
        dst[2 * t + WIN] = r[:, 128:]

    def halo(dst, h, is_v):
        r = pltpu.roll(dst[h + NB], 2, 1)
        if is_v:
            lane = lax.broadcasted_iota(jnp.int32, (D, 128), 1)
            r = jnp.where(lane < 2, dst[WIN - 1][:, 0:1], r)
        dst[h] = r

    def stage_q(t):
        r = proj(0, t)
        Q[(2 * t) & 3] = r[:, :128]
        Q[(2 * t + 1) & 3] = r[:, 128:]

    def stage_attn(t):
        lane = lax.broadcasted_iota(jnp.int32, (8, 128), 1)
        for b in range(2):
            j = 2 * t + b
            for g in range(4):
                acc = [None] * WIN
                for d in range(DH):
                    r = slice(g * 256 + d * 8, g * 256 + d * 8 + 8)
                    q = Q[j & 3, r, :]
                    for w in range(WIN):
                        p = q * KB[j + WIN - 1 - w, r, :]
                        acc[w] = p if d == 0 else acc[w] + p
                lg = [acc[w] * (DH ** -0.5) for w in range(WIN)]
                lg = [lg[0]] + [jnp.where((lane >= 2) | (j >= w), lg[w], -1e9) for w in range(1, WIN)]
                mx = lg[0]
                for w in range(1, WIN):
                    mx = jnp.maximum(mx, lg[w])
                e = [jnp.exp(l - mx) for l in lg]
                inv = 1.0 / sum(e[1:], e[0])
                a = [v * inv for v in e]
                for d in range(0, DH, 2):
                    o = []
                    for dd in (d, d + 1):
                        r = slice(g * 256 + dd * 8, g * 256 + dd * 8 + 8)
                        s = a[0] * VB[j + WIN - 1, r, :]
                        for w in range(1, WIN):
                            s = s + a[w] * VB[j + WIN - 1 - w, r, :]
                        o.append(s)
                    r0 = g * 256 + d * 8
                    O[j & 3, r0:r0 + 16, :] = jnp.concatenate(o, axis=0).astype(BF)

    def stage_wo(t):
        o = jnp.concatenate([O[(2 * t) & 3], O[(2 * t + 1) & 3]], axis=1)
        r = jnp.dot(WoT[...], o, preferred_element_type=F32)
        X[2 * t] += r[:, :128]
        X[2 * t + 1] += r[:, 128:]

    def stage_ln(t, twice):
        for b in range(2):
            H[2 * t + b] = _ln(X[2 * t + b], twice)

    def attn_main():
        def step(t):
            do = (lambda lo: lo <= t < lo + 8) if isinstance(t, int) else (lambda lo: True)
            if do(-1):
                stage_q(t + 1)
            if do(0):
                stage_attn(t)
            if do(1):
                stage_wo(t - 1)
            if do(2):
                stage_ln(t - 2, True)
        for t in (-1, 0, 1):
            step(t)
        loop(7, step, lo=2)
        for t in (7, 8, 9):
            step(t)

    def mix1(f):
        w = jnp.concatenate(
            [jnp.concatenate([_perm_rows(w1_u, 4 * f + c, j) for j in range(NB)], axis=0) for c in range(4)], axis=1)
        h = jnp.concatenate([H[j] for j in range(NB)], axis=1)
        cols = pl.ds(pl.multiple_of(f * 512, 512), 512)
        r = jnp.dot(h, w, preferred_element_type=F32) + B1[0:1, cols]
        U[:, cols] = _gelu(r).astype(BF)

    def w2_tile(t):
        return jnp.concatenate(
            [jnp.concatenate([_perm_rows(w2t_u, c, 2 * t + b) for c in range(F // 128)], axis=1) for b in range(2)],
            axis=0)

    def mix2(t):
        r = lax.dot_general(U[...], w2_tile(t), NT, preferred_element_type=F32)
        for b in range(2):
            X[2 * t + b] += r[:, b * 128:(b + 1) * 128] + B2[2 * t + b][0:1, :]

    def out_copy(c, slot):
        return pltpu.make_async_copy(xs.at[c], out_h.at[:, pl.ds(pl.multiple_of(c * 128, 128), 128)], sems.at[8 + slot])

    def mix2_final(m):
        rows = pl.ds(pl.multiple_of(m * 256, 256), 256)
        u = U[rows, :]
        for t in range(8):
            r = lax.dot_general(u, w2_tile(t), NT, preferred_element_type=F32)
            for b in range(2):
                j = 2 * t + b
                y = (X[j, rows, :] + (r[:, b * 128:(b + 1) * 128] + B2[j][0:1, :])).astype(BF)
                for c in range(2):
                    xs_u[2 * m + c, pl.ds(j, 64, stride=NB), :] = pltpu.bitcast(y[c * 128:(c + 1) * 128, :].T, U32)
        for c in range(2):
            out_copy(2 * m + c, 2 * m + c).start()

    wait(cp_w[1])
    loop(8, lambda k: prep_w(1, k))
    wait(cp_x)
    prep_x(0)
    prep_x(1)
    wait(cp_w[2])

    def k1(t):
        proj_kv(1, KB, t)
        prep_w(2, t)
        if t is not LAST:
            prep_x(2 * t + 2)
            prep_x(2 * t + 3)
    LAST = 7
    loop(7, k1)
    k1(LAST)
    wait(cp_w[0] + cp_wo)

    def v1(t):
        proj_kv(2, VB, t)
        prep_w(0, t)
        prep_wo(t)
        halo(KB, jnp.minimum(t, WIN - 2), False)
    loop(8, v1)
    loop(WIN - 1, lambda h: halo(VB, h, True))
    attn_main()
    wait(cp_w1 + cp_w2)

    def m1(f):
        mix1(f)
        for c in range(4):
            prep_w2(4 * f + c)
    loop(7, m1)
    mix2(0)

    def m2(t):
        mix2(t)
        stage_ln(t - 1, False)
    loop(8, m2, lo=1)

    proj_kv(1, KB, 0)
    stage_ln(7, False)
    loop(8, lambda t: proj_kv(1, KB, t), lo=1)

    def v2(t):
        proj_kv(2, VB, t)
        halo(KB, jnp.minimum(t, WIN - 2), False)
    loop(8, v2)
    loop(WIN - 1, lambda h: halo(VB, h, True))
    attn_main()
    loop(7, mix1)
    loop(4, mix2_final)
    for c in range(8):
        out_copy(c, c).wait()


@jax.jit
def pallas_interleave_layers__sliding_local_dilated__mixer_token_mlp__prompt_kernel(
    A_x, A_wqkv, A_wo, B_x, B_w1, B_b1, B_w2, B_b2):
    hbm = pl.BlockSpec(memory_space=pl.ANY)
    vm = pl.BlockSpec(memory_space=pltpu.VMEM)
    V = pltpu.VMEM
    out = pl.pallas_call(
        _kernel,
        out_shape=jax.ShapeDtypeStruct((S, D), BF),
        in_specs=[hbm, hbm, hbm, hbm, vm, hbm, vm],
        out_specs=hbm,
        scratch_shapes=[
            V((9, S // 2, 128), U32),
            V((24, D, 128), BF),
            V((D, D), BF),
            V((F // 128, S, 128), BF),
            V((F, S), BF),
            V((NB, D, 128), F32),
            V((NB, D, 128), BF),
            V((3, D, D), BF),
            V((D, D), BF),
            V((F // 128, S // 2, 128), U32),
            V((NB + WIN - 1, D, 128), F32),
            V((NB + WIN - 1, D, 128), F32),
            V((4, D, 128), F32),
            V((4, D, 128), BF),
            V((D, F), BF),
            V((D, 128), F32),
            V((8, F), F32),
            V((NB, 8, 128), F32),
            pltpu.SemaphoreType.DMA((16,)),
        ],
        compiler_params=pltpu.CompilerParams(vmem_limit_bytes=126 * 2**20),
    )(A_x.reshape(S, D), A_wqkv, A_wo, B_w1, B_b1, B_w2, B_b2)
    return out.reshape(1, S, D)
```

```python
import jax
import jax.numpy as jnp
from jax import lax
import jax.experimental.pallas as pl
import jax.experimental.pallas.tpu as pltpu

S, D, F = 2048, 1024, 3584
NH, DH, WIN = 32, 32, 8
NB = S // 128
EPS = 1e-5
BF, F32, U32 = jnp.bfloat16, jnp.float32, jnp.uint32
NT = (((1,), (1,)), ((), ()))


def _perm_rows(ref_u32, lead, j):
    return pltpu.bitcast(ref_u32[lead, pl.ds(j, 64, stride=NB), :], BF)


def _ln(x, twice):
    m = jnp.mean(x, axis=0, keepdims=True)
    c = x - m
    v = jnp.mean(c * c, axis=0, keepdims=True)
    r = lax.rsqrt(v + EPS)
    if twice:
        r = r * lax.rsqrt(v * r * r + EPS)
    return c * r


def _pk(x):
    return pltpu.bitcast(x.astype(BF), U32)


def _up(x):
    return pltpu.bitcast(x, BF)


def _acomb(a11, a12, a21, a22):
    return [a11 + a22, a21 + a22, a11, a22, a11 + a12, a21 - a11, a12 - a22]


def _bcomb(b11, b12, b21, b22):
    return [b11 + b22, b11, b12 - b22, b21 - b11, b22, b11 + b12, b21 + b22]


def _bcomb_lazy(load):
    f = lambda k, n: load(k, n).astype(F32)
    tab = [lambda: f(0, 0) + f(1, 1), lambda: load(0, 0), lambda: f(0, 1) - f(1, 1), lambda: f(1, 0) - f(0, 0),
           lambda: load(1, 1), lambda: f(0, 0) + f(0, 1), lambda: f(1, 0) + f(1, 1)]
    return lambda i: tab[i]().astype(BF)


def _strassen(a, b, sink, dims=(((1,), (0,)), ((), ()))):
    m = lambda i: lax.dot_general(a(i), b(i), dims, preferred_element_type=F32)
    m3, m5 = m(2), m(4)
    sink(0, 1, m3 + m5)
    m1 = m(0)
    p, q = m1 - m5, m1 + m3
    m2 = m(1)
    sink(1, 1, (q - m2) + m(5))
    m4 = m(3)
    sink(1, 0, m2 + m4)
    sink(0, 0, (p + m4) + m(6))


def _gelu(x):
    return 0.5 * x * (1.0 + jnp.tanh(0.7978845608028654 * (x + 0.044715 * x * x * x)))


def _kernel(x_h, wqkv_h, wo_h, w1_h, b1_ref, w2_h, b2_ref, out_h,
            xs_u, wraw, w1_u, w2raw, X, H, WT, w2t_u, KB, VB, Q, O, U, st, B1, B2, sems):
    xs, w1s = xs_u.bitcast(BF), w1_u.bitcast(BF)
    HALF = [slice(0, D // 2), slice(D // 2, D)]

    def col_copies(src, dst, lo, hi, sem):
        return [pltpu.make_async_copy(src.at[:, pl.ds(c * 128, 128)], dst.at[c], sems.at[sem])
                for c in range(lo, hi)]

    cp_x = col_copies(x_h, xs, 0, 8, 0)
    cp_w = [col_copies(wqkv_h, wraw, 8 * p, 8 * p + 8, 1 + p) for p in range(3)]
    cp_wo = col_copies(wo_h, wraw.at[pl.ds(24, 8)], 0, 8, 4)
    cp_w1 = col_copies(w1_h, w1s, 0, F // 128, 5)
    def cp_w2(f):
        return pltpu.make_async_copy(w2_h.at[pl.ds(pl.multiple_of(f * 512, 512), 512)], w2raw.at[f & 1], sems.at[6 + (f & 1)])
    for cp in cp_w[1] + cp_x + cp_w[2] + cp_w[0] + cp_wo + cp_w1 + [cp_w2(0)]:
        cp.start()

    def wait(cps):
        for cp in cps:
            cp.wait()

    def prep_w(part, kc):
        cols = pl.ds(pl.multiple_of(kc * 128, 128), 128)
        for k in range(2):
            rows = pl.ds(pl.multiple_of(kc * 128 + k * 512, 128), 128)
            for c in range(8):
                st[k, c * 128:(c + 1) * 128, :] = wraw[part * 8 + c, rows, :].astype(F32).T
        for g in range(2):
            for d in range(0, DH, 2):
                quad = [jnp.concatenate([st[k, pl.ds((2 * r + g) * 256 + dd, 8, stride=DH), :] for dd in (d, d + 1)], axis=0)
                        for r in range(2) for k in range(2)]
                for i, a in enumerate(_acomb(*quad)):
                    WT[part, i, g * 128 + d * 4:g * 128 + d * 4 + 8, cols] = _pk(a)

    def prep_wo(c):
        for r in range(2):
            st[2 + r] = wraw[24 + 4 * r + c].astype(F32)
        for kk in range(4):
            quad = []
            for r in range(2):
                for k in range(2):
                    g, d0 = 2 * k + kk // 2, (kk % 2) * 16
                    quad.append(jnp.concatenate(
                        [st[2 + r, pl.ds(g * 256 + d0 + d, 8, stride=DH), :] for d in range(16)], axis=0).T)
            for i, a in enumerate(_acomb(*quad)):
                WT[3, i, pl.ds(pl.multiple_of(c * 64, 64), 64), kk * 128:(kk + 1) * 128] = _pk(a)

    def prep_w2(f):
        for c in range(4):
            for j in range(NB):
                w2t_u[4 * f + c, j * 64:(j + 1) * 64, :] = pltpu.bitcast(
                    w2raw[f & 1, c * 128:(c + 1) * 128, j * 128:(j + 1) * 128].T, U32)

    def put_h(t, x0, x1, mixer):
        h0, h1 = _ln(x0, mixer), _ln(x1, mixer)
        comb = _acomb if mixer else _bcomb
        for i, a in enumerate(comb(h0[HALF[0]], h1[HALF[0]], h0[HALF[1]], h1[HALF[1]])):
            H[i, t] = _pk(a)

    def prep_x(t):
        xt = []
        for j in (2 * t, 2 * t + 1):
            xt.append(jnp.concatenate([_perm_rows(xs_u, c, j).T for c in range(8)], axis=0).astype(F32))
            X[j] = xt[-1]
            B2[j] = _perm_rows(xs_u, 8, j).T[0:16, :].astype(F32)[0:8, :]
        put_h(t, xt[0], xt[1], False)

    B1[...] = jnp.broadcast_to(b1_ref[...].astype(F32).reshape(1, F), (8, F))
    b2 = b2_ref[...].astype(F32).reshape(1, S)
    for c in range(NB):
        xs_u[8, c * 64:(c + 1) * 64, :] = pltpu.bitcast(
            jnp.broadcast_to(b2[:, c * 128:(c + 1) * 128], (128, 128)).T.astype(BF), U32)

    def loop(n, fn, lo=0):
        def body(i, c):
            fn(i)
            return c
        lax.fori_loop(lo, n, body, 0)

    def proj(part, t, sink):
        _strassen(lambda i: _up(WT[part, i]), lambda i: _up(H[i, t]), sink)

    def proj_kv(part, dst, t):
        def sink(r, n, v):
            dst[2 * t + n + WIN - 1, HALF[r], :] = v
        proj(part, t, sink)

    def halo(dst, h, is_v):
        r = pltpu.roll(dst[h + NB], 2, 1)
        if is_v:
            lane = lax.broadcasted_iota(jnp.int32, (D, 128), 1)
            r = jnp.where(lane < 2, dst[WIN - 1][:, 0:1], r)
        dst[h] = r

    def stage_q(t):
        def sink(r, n, v):
            Q[(2 * t + n) & 3, HALF[r], :] = v
        proj(0, t, sink)

    def stage_attn(t):
        lane = lax.broadcasted_iota(jnp.int32, (8, 128), 1)

        def probs(j, g):
            acc = [None] * WIN
            for d in range(DH):
                r = slice(g * 256 + d * 8, g * 256 + d * 8 + 8)
                q = Q[j & 3, r, :]
                for w in range(WIN):
                    p = q * KB[j + WIN - 1 - w, r, :]
                    acc[w] = p if d == 0 else acc[w] + p
            lg = [acc[w] * (DH ** -0.5) for w in range(WIN)]
            lg = [lg[0]] + [jnp.where((lane >= 2) | (j >= w), lg[w], -1e9) for w in range(1, WIN)]
            mx = lg[0]
            for w in range(1, WIN):
                mx = jnp.maximum(mx, lg[w])
            e = [jnp.exp(l - mx) for l in lg]
            inv = 1.0 / sum(e[1:], e[0])
            return [v * inv for v in e]

        for g in range(2):
            quads = [(2 * t + n, 2 * k + g) for k in range(2) for n in range(2)]
            pr = [probs(j, gg) for j, gg in quads]
            for d in range(0, DH, 2):
                o = []
                for (j, gg), a in zip(quads, pr):
                    two = []
                    for dd in (d, d + 1):
                        r = slice(gg * 256 + dd * 8, gg * 256 + dd * 8 + 8)
                        s = a[0] * VB[j + WIN - 1, r, :]
                        for w in range(1, WIN):
                            s = s + a[w] * VB[j + WIN - 1 - w, r, :]
                        two.append(s)
                    o.append(jnp.concatenate(two, axis=0))
                for i, v in enumerate(_bcomb(*o)):
                    O[i, t & 1, g * 128 + d * 4:g * 128 + d * 4 + 8, :] = _pk(v)

    def stage_wo(t):
        def sink(r, n, v):
            X[2 * t + n, HALF[r], :] += v
        _strassen(lambda i: _up(WT[3, i]), lambda i: _up(O[i, t & 1]), sink)

    def stage_ln(t, mixer):
        put_h(t, X[2 * t], X[2 * t + 1], mixer)

    def attn_main():
        def step(t):
            do = (lambda lo: lo <= t < lo + 8) if isinstance(t, int) else (lambda lo: True)
            if do(2):
                stage_ln(t - 2, True)
            if do(1):
                stage_wo(t - 1)
            if do(0):
                stage_attn(t)
            if do(-1):
                stage_q(t + 1)
        for t in (-1, 0, 1):
            step(t)
        loop(7, step, lo=2)
        for t in (7, 8, 9):
            step(t)

    def mix1(f):
        def w(k, n):
            return jnp.concatenate(
                [jnp.concatenate([_perm_rows(w1_u, 4 * f + 2 * n + c, 2 * t + k) for t in range(8)], axis=0)
                 for c in range(2)], axis=1)
        u = {}

        def sink(r, n, v):
            u[r, n] = _gelu(v + B1[0:1, pl.ds(pl.multiple_of(f * 512 + n * 256, 256), 256)])
        _strassen(lambda i: jnp.concatenate([_up(H[i, t]) for t in range(8)], axis=1), _bcomb_lazy(w), sink)
        for i, a in enumerate(_acomb(u[0, 0], u[0, 1], u[1, 0], u[1, 1])):
            U[i, :, pl.ds(pl.multiple_of(f * 256, 256), 256)] = _pk(a)

    def w2_tile(t):
        return _bcomb_lazy(lambda k, n: jnp.concatenate(
            [_perm_rows(w2t_u, 4 * f + 2 * k + c, 2 * t + n) for f in range(7) for c in range(2)], axis=1))

    def mix2(t):
        def sink(r, n, v):
            X[2 * t + n, HALF[r], :] += v + B2[2 * t + n][0:1, :]
        _strassen(lambda i: _up(U[i]), w2_tile(t), sink, NT)

    def out_copy(c, slot):
        return pltpu.make_async_copy(xs.at[c], out_h.at[:, pl.ds(pl.multiple_of(c * 128, 128), 128)], sems.at[8 + slot])

    def mix2_final(m):
        def tile(t):
            def sink(r, n, v):
                j = 2 * t + n
                rows = pl.ds(pl.multiple_of(r * 512 + m * 256, 256), 256)
                y = (X[j, rows, :] + (v + B2[j][0:1, :])).astype(BF)
                for c in range(2):
                    xs_u[4 * r + 2 * m + c, pl.ds(j, 64, stride=NB), :] = pltpu.bitcast(y[c * 128:(c + 1) * 128, :].T, U32)
            _strassen(lambda i: _up(U[i, pl.ds(pl.multiple_of(m * 128, 128), 128), :]), w2_tile(t), sink, NT)
        loop(8, tile)
        for c in (0, 1, 4, 5):
            out_copy(2 * m + c, 2 * m + c).start()

    wait(cp_w[1])
    loop(4, lambda k: prep_w(1, k))
    wait(cp_x)
    prep_x(0)
    wait(cp_w[2])

    def k1(t):
        proj_kv(1, KB, t)
        prep_w(2, t)
        prep_x(t + 1)
    loop(4, k1)
    wait(cp_w[0])

    def k2(t):
        proj_kv(1, KB, t)
        prep_w(0, t - 4)
        prep_x(jnp.minimum(t + 1, 7))
    loop(8, k2, lo=4)
    wait(cp_wo)

    def v1(t):
        proj_kv(2, VB, t)
        prep_wo(t)
        halo(KB, t, False)
    loop(4, v1)

    def v2(t):
        proj_kv(2, VB, t)
        halo(KB, jnp.minimum(t, WIN - 2), False)
    loop(8, v2, lo=4)
    loop(WIN - 1, lambda h: halo(VB, h, True))
    attn_main()
    wait(cp_w1)

    def m1(f):
        @pl.when(f < 6)
        def _():
            cp_w2(f + 1).start()
        cp_w2(f).wait()
        mix1(f)
        prep_w2(f)
    loop(7, m1)
    mix2(0)

    def m2(t):
        stage_ln(t - 1, False)
        mix2(t)
    loop(8, m2, lo=1)

    proj_kv(1, KB, 0)
    stage_ln(7, False)
    loop(8, lambda t: proj_kv(1, KB, t), lo=1)

    loop(8, v2)
    loop(WIN - 1, lambda h: halo(VB, h, True))
    attn_main()
    loop(7, mix1)
    loop(2, mix2_final)
    for c in range(8):
        out_copy(c, c).wait()


@jax.jit
def pallas_interleave_layers__sliding_local_dilated__mixer_token_mlp__prompt_kernel(
    A_x, A_wqkv, A_wo, B_x, B_w1, B_b1, B_w2, B_b2):
    hbm = pl.BlockSpec(memory_space=pl.ANY)
    vm = pl.BlockSpec(memory_space=pltpu.VMEM)
    V = pltpu.VMEM
    out = pl.pallas_call(
        _kernel,
        out_shape=jax.ShapeDtypeStruct((S, D), BF),
        in_specs=[hbm, hbm, hbm, hbm, vm, hbm, vm],
        out_specs=hbm,
        scratch_shapes=[
            V((9, S // 2, 128), U32),
            V((32, D, 128), BF),
            V((F // 128, S // 2, 128), U32),
            V((2, 512, S), BF),
            V((NB, D, 128), F32),
            V((7, 8, D // 4, 128), U32),
            V((4, 7, D // 4, D // 2), U32),
            V((F // 128, S // 2, 128), U32),
            V((NB + WIN - 1, D, 128), F32),
            V((NB + WIN - 1, D, 128), F32),
            V((4, D, 128), F32),
            V((7, 2, D // 4, 128), U32),
            V((7, D // 4, F // 2), U32),
            V((4, D, 128), F32),
            V((8, F), F32),
            V((NB, 8, 128), F32),
            pltpu.SemaphoreType.DMA((16,)),
        ],
        compiler_params=pltpu.CompilerParams(vmem_limit_bytes=126 * 2**20),
    )(A_x.reshape(S, D), A_wqkv, A_wo, B_w1, B_b1, B_w2, B_b2)
    return out.reshape(1, S, D)
```

```python
import jax
import jax.numpy as jnp
from jax import lax
import jax.experimental.pallas as pl
import jax.experimental.pallas.tpu as pltpu

S, D, F = 2048, 1024, 3584
NH, DH, WIN = 32, 32, 8
NB = S // 128
EPS = 1e-5
PAD = 40
BF, F32, U32 = jnp.bfloat16, jnp.float32, jnp.uint32
NT = (((1,), (1,)), ((), ()))


def _perm_rows(ref_u32, lead, j):
    return pltpu.bitcast(ref_u32[lead, pl.ds(j, 64, stride=NB), :], BF)


def _pk(x):
    return pltpu.bitcast(x.astype(BF), U32)


def _up(x):
    return pltpu.bitcast(x, BF)


def _acomb(a11, a12, a21, a22):
    return [a11 + a22, a21 + a22, a11, a22, a11 + a12, a21 - a11, a12 - a22]


def _bcomb(b11, b12, b21, b22):
    return [b11 + b22, b11, b12 - b22, b21 - b11, b22, b11 + b12, b21 + b22]


def _bcomb_lazy(load):
    f = lambda k, n: load(k, n).astype(F32)
    tab = [lambda: f(0, 0) + f(1, 1), lambda: load(0, 0), lambda: f(0, 1) - f(1, 1), lambda: f(1, 0) - f(0, 0),
           lambda: load(1, 1), lambda: f(0, 0) + f(0, 1), lambda: f(1, 0) + f(1, 1)]
    return lambda i: tab[i]().astype(BF)


class _Side:
    jobs = []


def _together(main, ticks, *jobs):
    _Side.jobs = [(g, -(-n // ticks)) for g, n in jobs]
    main()
    for g, _ in jobs:
        for _ in g:
            pass
    _Side.jobs = []


def _strassen(a, b, sink, dims=(((1,), (0,)), ((), ()))):
    def m(i):
        for g, n in _Side.jobs:
            for _ in range(n):
                next(g, None)
        return lax.dot_general(a(i), b(i), dims, preferred_element_type=F32)
    m3, m5 = m(2), m(4)
    sink(0, 1, m3 + m5)
    m1 = m(0)
    p, q = m1 - m5, m1 + m3
    m2 = m(1)
    sink(1, 1, (q - m2) + m(5))
    m4 = m(3)
    sink(1, 0, m2 + m4)
    sink(0, 0, (p + m4) + m(6))


def _gelu(x):
    return 0.5 * x * (1.0 + jnp.tanh(0.7978845608028654 * (x + 0.044715 * x * x * x)))


def _kernel(x_h, wqkv_h, wo_h, w1_h, b1_ref, w2_h, b2_ref, out_h,
            xs_u, wraw, w1_u, w2raw, X, H, WT, w2t_u, KB, VB, Q, O, U, st, B1, B2, sems):
    xs, w1s = xs_u.bitcast(BF), w1_u.bitcast(BF)
    HALF = [slice(0, D // 2), slice(D // 2, D)]

    def col_copies(src, dst, lo, hi, sem):
        return [pltpu.make_async_copy(src.at[:, pl.ds(c * 128, 128)], dst.at[c], sems.at[sem])
                for c in range(lo, hi)]

    cp_x = col_copies(x_h, xs, 0, 8, 0)
    cp_w = [col_copies(wqkv_h, wraw, 8 * p, 8 * p + 8, 1 + p) for p in range(3)]
    cp_wo = col_copies(wo_h, wraw.at[pl.ds(24, 8)], 0, 8, 4)
    cp_w1 = col_copies(w1_h, w1s, 0, F // 128, 5)
    def cp_w2(f):
        return pltpu.make_async_copy(w2_h.at[pl.ds(pl.multiple_of(f * 512, 512), 512)], w2raw.at[f & 1], sems.at[6 + (f & 1)])
    for cp in cp_w[1] + cp_x + cp_w[2] + cp_w[0] + cp_wo + cp_w1 + [cp_w2(0)]:
        cp.start()

    def wait(cps):
        for cp in cps:
            cp.wait()

    def prep_w(part, kc):
        cols = pl.ds(pl.multiple_of(kc * 128, 128), 128)
        for k in range(2):
            rows = pl.ds(pl.multiple_of(kc * 128 + k * 512, 128), 128)
            for c in range(8):
                blk = wraw[part * 8 + c, rows, :].astype(F32).T
                for h in range(4):
                    st[k, (4 * c + h) * PAD:(4 * c + h) * PAD + DH, :] = blk[h * DH:(h + 1) * DH]
                yield
        for g in range(2):
            for d in range(0, DH, 2):
                quad = [jnp.concatenate([st[k, pl.ds((2 * r + g) * 8 * PAD + dd, 8, stride=PAD), :] for dd in (d, d + 1)], axis=0)
                        for r in range(2) for k in range(2)]
                for i, a in enumerate(_acomb(*quad)):
                    WT[part, i, g * 128 + d * 4:g * 128 + d * 4 + 8, cols] = _pk(a)
                yield

    def prep_wo(c):
        for r in range(2):
            for h in range(NH):
                st[2 + r, h * PAD:h * PAD + DH, :] = wraw[24 + 4 * r + c, h * DH:(h + 1) * DH, :].astype(F32)
        for kk in range(4):
            quad = []
            for r in range(2):
                for k in range(2):
                    g, d0 = 2 * k + kk // 2, (kk % 2) * 16
                    quad.append(jnp.concatenate(
                        [st[2 + r, pl.ds(g * 8 * PAD + d0 + d, 8, stride=PAD), :] for d in range(16)], axis=0).T)
                    yield
            for i, a in enumerate(_acomb(*quad)):
                WT[3, i, pl.ds(pl.multiple_of(c * 64, 64), 64), kk * 128:(kk + 1) * 128] = _pk(a)

    def prep_w2(f):
        for c in range(4):
            for j in range(NB):
                w2t_u[4 * f + c, j * 64:(j + 1) * 64, :] = pltpu.bitcast(
                    w2raw[f & 1, c * 128:(c + 1) * 128, j * 128:(j + 1) * 128].T, U32)
                yield

    def put_h(t, mixer):
        stats = []
        for j in (2 * t, 2 * t + 1):
            chunks = [slice(c * 32, c * 32 + 32) for c in range(D // 32)]
            m = jnp.sum(sum(X[j, c, :] for c in chunks), axis=0, keepdims=True) * (1.0 / D)
            yield
            v = jnp.sum(sum(jnp.square(X[j, c, :] - m) for c in chunks), axis=0, keepdims=True) * (1.0 / D)
            r = lax.rsqrt(v + EPS)
            if mixer:
                r = r * lax.rsqrt(v * r * r + EPS)
            stats.append((m, r))
            yield
            yield
            yield
        comb = _acomb if mixer else _bcomb
        for c in range(D // 32):
            quad = [(X[2 * t + n, k * 512 + c * 16:k * 512 + c * 16 + 16, :] - stats[n][0]) * stats[n][1]
                    for k in range(2) for n in range(2)]
            for i, a in enumerate(comb(*quad)):
                H[i, t, c * 8:c * 8 + 8, :] = _pk(a)
            if c % 2:
                yield

    def prep_x(t):
        for j in (2 * t, 2 * t + 1):
            for c in range(8):
                X[j, c * 128:(c + 1) * 128, :] = _perm_rows(xs_u, c, j).T.astype(F32)
                yield
            B2[j] = _perm_rows(xs_u, 8, j).T[0:16, :].astype(F32)[0:8, :]
        yield from put_h(t, False)

    B1[...] = jnp.broadcast_to(b1_ref[...].astype(F32).reshape(1, F), (8, F))
    b2 = b2_ref[...].astype(F32).reshape(1, S)
    for c in range(NB):
        xs_u[8, c * 64:(c + 1) * 64, :] = pltpu.bitcast(
            jnp.broadcast_to(b2[:, c * 128:(c + 1) * 128], (128, 128)).T.astype(BF), U32)

    def loop(n, fn, lo=0):
        def body(i, c):
            fn(i)
            return c
        lax.fori_loop(lo, n, body, 0)

    def proj(part, t, sink):
        _strassen(lambda i: _up(WT[part, i]), lambda i: _up(H[i, t]), sink)

    def proj_kv(part, dst, t):
        def sink(r, n, v):
            dst[2 * t + n + WIN - 1, HALF[r], :] = v
        proj(part, t, sink)

    def halo(dst, h, is_v):
        r = pltpu.roll(dst[h + NB], 2, 1)
        if is_v:
            lane = lax.broadcasted_iota(jnp.int32, (D, 128), 1)
            r = jnp.where(lane < 2, dst[WIN - 1][:, 0:1], r)
        dst[h] = r

    def stage_q(t):
        def sink(r, n, v):
            Q[(2 * t + n) & 3, HALF[r], :] = v
        proj(0, t, sink)

    def stage_attn(t):
        lane = lax.broadcasted_iota(jnp.int32, (8, 128), 1)

        def logits(g):
            acc = [[None] * WIN, [None] * WIN]
            for d in range(DH):
                r = slice(g * 256 + d * 8, g * 256 + d * 8 + 8)
                q = [Q[(2 * t + n) & 3, r, :] for n in range(2)]
                for b in range(WIN + 1):
                    k = KB[2 * t + b, r, :]
                    for n in range(2):
                        w = n + WIN - 1 - b
                        if 0 <= w < WIN:
                            acc[n][w] = q[n] * k if d == 0 else acc[n][w] + q[n] * k
                if d % 4 == 3:
                    yield
            return acc

        def probs(j, acc):
            lg = [acc[w] * (DH ** -0.5) for w in range(WIN)]
            lg = [lg[0]] + [jnp.where((lane >= 2) | (j >= w), lg[w], -1e9) for w in range(1, WIN)]
            mx = lg[0]
            for w in range(1, WIN):
                mx = jnp.maximum(mx, lg[w])
            e = [jnp.exp(l - mx) for l in lg]
            inv = 1.0 / sum(e[1:], e[0])
            return [v * inv for v in e]

        for g in range(2):
            pr = []
            for k in range(2):
                accs = yield from logits(2 * k + g)
                pr.append([probs(2 * t + n, accs[n]) for n in range(2)])
            for d in range(0, DH, 2):
                o = []
                for k in range(2):
                    two = [[], []]
                    for dd in (d, d + 1):
                        r0 = (2 * k + g) * 256 + dd * 8
                        v = [VB[2 * t + b, r0:r0 + 8, :] for b in range(WIN + 1)]
                        for n in range(2):
                            two[n].append(sum((pr[k][n][w] * v[n + WIN - 1 - w] for w in range(1, WIN)),
                                              pr[k][n][0] * v[n + WIN - 1]))
                    o += [jnp.concatenate(x, axis=0) for x in two]
                for i, v in enumerate(_bcomb(*o)):
                    O[i, t & 1, g * 128 + d * 4:g * 128 + d * 4 + 8, :] = _pk(v)
                yield

    def stage_wo(t):
        def sink(r, n, v):
            X[2 * t + n, HALF[r], :] += v
        _strassen(lambda i: _up(WT[3, i]), lambda i: _up(O[i, t & 1]), sink)

    def stage_ln(t, mixer):
        return put_h(t, mixer), 24

    def attn_main():
        def step(t):
            do = (lambda lo: lo <= t < lo + 8) if isinstance(t, int) else (lambda lo: True)
            def main():
                if do(-1):
                    stage_q(t + 1)
                if do(1):
                    stage_wo(t - 1)
            ticks = 7 * (do(-1) + do(1))
            jobs = []
            if do(2):
                jobs.append((put_h(t - 2, True), 24 * max(ticks, 1) // 8))
            if do(0):
                jobs.append((stage_attn(t), 64))
            _together(main, max(ticks, 1), *jobs)
        for t in (-1, 0, 1):
            step(t)
        loop(7, step, lo=2)
        for t in (7, 8, 9):
            step(t)

    def mix1(f):
        def w(k, n):
            return jnp.concatenate(
                [jnp.concatenate([_perm_rows(w1_u, 4 * f + 2 * n + c, 2 * t + k) for t in range(8)], axis=0)
                 for c in range(2)], axis=1)
        u = {}

        def sink(r, n, v):
            u[r, n] = _gelu(v + B1[0:1, pl.ds(pl.multiple_of(f * 512 + n * 256, 256), 256)])
        _strassen(lambda i: jnp.concatenate([_up(H[i, t]) for t in range(8)], axis=1), _bcomb_lazy(w), sink)
        for i, a in enumerate(_acomb(u[0, 0], u[0, 1], u[1, 0], u[1, 1])):
            U[i, :, pl.ds(pl.multiple_of(f * 256, 256), 256)] = _pk(a)

    def w2_tile(t):
        return _bcomb_lazy(lambda k, n: jnp.concatenate(
            [_perm_rows(w2t_u, 4 * f + 2 * k + c, 2 * t + n) for f in range(7) for c in range(2)], axis=1))

    def mix2(t):
        def sink(r, n, v):
            X[2 * t + n, HALF[r], :] += v + B2[2 * t + n][0:1, :]
        _strassen(lambda i: _up(U[i]), w2_tile(t), sink, NT)

    def out_copy(c, slot):
        return pltpu.make_async_copy(xs.at[c], out_h.at[:, pl.ds(pl.multiple_of(c * 128, 128), 128)], sems.at[8 + slot])

    def mix2_final(m):
        def tile(t):
            def sink(r, n, v):
                j = 2 * t + n
                rows = HALF[r]
                y = (X[j, rows, :] + (v + B2[j][0:1, :])).astype(BF)
                for c in range(4):
                    xs_u[4 * r + c, pl.ds(j, 64, stride=NB), :] = pltpu.bitcast(y[c * 128:(c + 1) * 128, :].T, U32)
            _strassen(lambda i: _up(U[i]), w2_tile(t), sink, NT)
        loop(8, tile)
        for c in range(8):
            out_copy(c, c).start()

    wait(cp_w[1])
    loop(4, lambda k: _together(lambda: None, 1, (prep_w(1, k), 1)))
    wait(cp_x)
    _together(lambda: None, 1, (prep_x(0), 1))
    wait(cp_w[2])

    def k1(t):
        _together(lambda: proj_kv(1, KB, t), 7, (prep_w(2, t), 48), (prep_x(t + 1), 40))
    loop(4, k1)
    wait(cp_w[0])

    def k2(t):
        _together(lambda: proj_kv(1, KB, t), 7, (prep_x(t + 1), 40))
    loop(7, k2, lo=4)
    proj_kv(1, KB, 7)
    wait(cp_wo)

    def v_phase(first):
        def va(i):
            halo(KB, i, False)
            halo(KB, i + 3, False)
            _together(lambda: proj_kv(2, VB, jnp.where(i == 0, 0, i + 3)), 7, *([(prep_wo(i), 16)] if first else []))
        loop(4, va)

        def vb(i):
            halo(VB, i, True)
            halo(VB, i + 3, True)
            _together(lambda: proj_kv(2, VB, jnp.where(i == 0, 7, i)), 7, *([(prep_w(0, i), 48)] if first else []))
        loop(4, vb)

    v_phase(True)
    attn_main()
    wait(cp_w1)

    def m1(f):
        @pl.when(f < 6)
        def _():
            cp_w2(f + 1).start()
        cp_w2(f).wait()
        _together(lambda: mix1(f), 7, (prep_w2(f), 64))
    loop(7, m1)
    loop(7, mix2)
    _together(lambda: mix2(7), 7, stage_ln(0, False))

    loop(7, lambda t: _together(lambda: proj_kv(1, KB, t), 6, stage_ln(t + 1, False)))
    proj_kv(1, KB, 7)
    v_phase(False)
    attn_main()
    loop(7, mix1)
    mix2_final(0)
    for c in range(8):
        out_copy(c, c).wait()


@jax.jit
def pallas_interleave_layers__sliding_local_dilated__mixer_token_mlp__prompt_kernel(
    A_x, A_wqkv, A_wo, B_x, B_w1, B_b1, B_w2, B_b2):
    hbm = pl.BlockSpec(memory_space=pl.ANY)
    vm = pl.BlockSpec(memory_space=pltpu.VMEM)
    V = pltpu.VMEM
    out = pl.pallas_call(
        _kernel,
        out_shape=jax.ShapeDtypeStruct((S, D), BF),
        in_specs=[hbm, hbm, hbm, hbm, vm, hbm, vm],
        out_specs=hbm,
        scratch_shapes=[
            V((9, S // 2, 128), U32),
            V((32, D, 128), BF),
            V((F // 128, S // 2, 128), U32),
            V((2, 512, S), BF),
            V((NB, D, 128), F32),
            V((7, 8, D // 4, 128), U32),
            V((4, 7, D // 4, D // 2), U32),
            V((F // 128, S // 2, 128), U32),
            V((NB + WIN - 1, D, 128), F32),
            V((NB + WIN - 1, D, 128), F32),
            V((4, D, 128), F32),
            V((7, 2, D // 4, 128), U32),
            V((7, D // 4, F // 2), U32),
            V((4, (NH + 1) * PAD, 128), F32),
            V((8, F), F32),
            V((NB, 8, 128), F32),
            pltpu.SemaphoreType.DMA((16,)),
        ],
        compiler_params=pltpu.CompilerParams(vmem_limit_bytes=126 * 2**20),
    )(A_x.reshape(S, D), A_wqkv, A_wo, B_w1, B_b1, B_w2, B_b2)
    return out.reshape(1, S, D)
```
